```python
import os as _os
_os.environ.setdefault("JAX_PLATFORMS", "cpu")
import jax
import jax.numpy as jnp

def _softmax(x, axis=-1):
    return jax.nn.softmax(x, axis=axis)
def _gelu(x):
    return jax.nn.gelu(x, approximate=True)
def _silu(x):
    return jax.nn.silu(x)
def _sigmoid(x):
    return jax.nn.sigmoid(x)
def _layernorm(x, axis=-1, eps=1e-5):
    m = jnp.mean(x, axis=axis, keepdims=True)
    v = jnp.var(x, axis=axis, keepdims=True)
    return (x - m) / jnp.sqrt(v + eps)
def _scatter_add(tgt, idx, src, axis=0):
    return tgt.at[idx].add(src)
def _segment_sum(src, seg, n):
    return jax.ops.segment_sum(src, seg, n)
class _Rng:
    def __init__(self, key):
        self._k = key
    def _next(self):
        self._k, sub = jax.random.split(self._k)
        return sub
    def normal(self, shape):
        return jax.random.normal(self._next(), shape, dtype=jnp.bfloat16)
    def randint(self, lo, hi, shape):
        return jax.random.randint(self._next(), shape, lo, hi, dtype=jnp.int32)
    def uniform(self, shape, lo=0.0, hi=1.0):
        return jax.random.uniform(self._next(), shape, jnp.bfloat16, lo, hi)
    def permutation(self, n):
        return jax.random.permutation(self._next(), n)


kernel_name = 'standalone__glu_gated_bilinear__prompt'

def setup_inputs():
    _rng = _Rng(jax.random.key(int.from_bytes(__import__("os").urandom(4), "little")))
    _w = (lambda a: (lambda t: t.astype(jnp.bfloat16) if jnp.issubdtype(t.dtype, jnp.floating) else t)(jnp.asarray(a)))
    B, S, D, F = 1, 2048, 640, 1728
    return {
        "x": _w((lambda *s: _rng.normal(s) * 0.05)(B, S, D)),
        "w_gate": _w((lambda *s: _rng.normal(s) * 0.05)(D, F) * (D ** -0.5)),
        "w_up": _w((lambda *s: _rng.normal(s) * 0.05)(D, F) * (D ** -0.5)),
        "w_down": _w((lambda *s: _rng.normal(s) * 0.05)(F, D) * (F ** -0.5)),
    }

def reference(x, w_gate, w_up, w_down):
    g = jnp.einsum("bsd,df->bsf", x, w_gate)
    u = jnp.einsum("bsd,df->bsf", x, w_up)
    h = g * u
    return jnp.einsum("bsf,fd->bsd", h, w_down)
```

```python
import functools
import jax
import jax.numpy as jnp
from jax import lax
import jax.experimental.pallas as pl
import jax.experimental.pallas.tpu as pltpu

NT = (((1,), (1,)), ((), ()))
f32 = jnp.float32
bf16 = jnp.bfloat16

def make(tm=256, fchunks=(256, 512, 896), loop=True):
    def kern(x_hbm, wg_hbm, wu_hbm, wd_hbm, o_hbm, x_v, wg_v, wu_v, wt_v, wd_v, o_v, sem, sem_o):
        S, D = x_hbm.shape
        F = wg_hbm.shape[0]
        FM = F // 128 * 128
        FT = F - FM
        nm = S // tm
        assert sum(fchunks) == FM
        offs = [sum(fchunks[:i]) for i in range(len(fchunks))]
        nf = len(fchunks)
        k = iter(range(1000))
        cp = lambda a, b: pltpu.make_async_copy(a, b, sem.at[next(k)])
        x0 = cp(x_hbm.at[pl.ds(0, tm)], x_v.at[pl.ds(0, tm)])
        g_cp, u_cp = [], []
        for o, n in zip(offs, fchunks):
            g_cp.append(cp(wg_hbm.at[pl.ds(o, n)], wg_v.at[pl.ds(o, n)]))
            u_cp.append(cp(wu_hbm.at[pl.ds(o, n)], wu_v.at[pl.ds(o, n)]))
        tg_cp = cp(wg_hbm.at[pl.ds(FM, FT)], wt_v.at[pl.ds(0, FT)])
        tu_cp = cp(wu_hbm.at[pl.ds(FM, FT)], wt_v.at[pl.ds(FT, FT)])
        d_cp = cp(wd_hbm, wd_v.at[pl.ds(0, F)])
        xr = cp(x_hbm.at[pl.ds(tm, S - tm)], x_v.at[pl.ds(tm, S - tm)])
        x0.start()
        for j in range(nf):
            g_cp[j].start(); u_cp[j].start()
        tg_cp.start(); tu_cp.start()
        d_cp.start()
        xr.start()
        wd_v[pl.ds(F, 128 - FT), :] = jnp.zeros((128 - FT, D), bf16)

        def ffn(rows, first):
            hs = []
            for j, (o, n) in enumerate(zip(offs, fchunks) if first else [(0, FM)]):
                if first:
                    g_cp[j].wait(); u_cp[j].wait()
                    if j == nf - 1:
                        tg_cp.wait(); tu_cp.wait()
                x = x_v[rows, :]
                g = lax.dot_general(x, wg_v[pl.ds(o, n), :], NT, preferred_element_type=f32)
                u = lax.dot_general(x, wu_v[pl.ds(o, n), :], NT, preferred_element_type=f32)
                hs.append((g * u).astype(bf16))
            t = lax.dot_general(x, wt_v[...], NT, preferred_element_type=f32)
            ht = t * pltpu.roll(t, FT, 1)
            lane = lax.broadcasted_iota(jnp.int32, ht.shape, 1)
            hs.append(jnp.where(lane < FT, ht, 0.0).astype(bf16))
            h = jnp.concatenate(hs, axis=1)
            if first: d_cp.wait()
            o_v[rows, :] = jnp.dot(h, wd_v[...], preferred_element_type=f32).astype(bf16)

        def out_cp(i):
            r = pl.ds(pl.multiple_of(i * tm, tm), tm)
            return pltpu.make_async_copy(o_v.at[r], o_hbm.at[r], sem_o.at[i])

        x0.wait()
        ffn(pl.ds(0, tm), True)
        out_cp(0).start()
        xr.wait()
        if loop:
            def body(i, c):
                r = pl.ds(pl.multiple_of(i * tm, tm), tm)
                ffn(r, False)
                out_cp(i).start()
                return c
            lax.fori_loop(1, nm, body, 0)
        else:
            for i in range(1, nm):
                ffn(pl.ds(i * tm, tm), False)
                out_cp(i).start()
        for i in range(nm):
            pltpu.make_async_copy(o_v.at[pl.ds(i * tm, tm)], o_hbm.at[pl.ds(i * tm, tm)], sem_o.at[i]).wait()

    def fn(x, w_gate, w_up, w_down):
        B, S, D = x.shape
        F = w_gate.shape[1]
        x2 = x.reshape(B * S, D)
        nm = B * S // tm
        FM = F // 128 * 128
        out = pl.pallas_call(
            kern,
            in_specs=[pl.BlockSpec(memory_space=pl.ANY)] * 4,
            out_specs=pl.BlockSpec(memory_space=pl.ANY),
            out_shape=jax.ShapeDtypeStruct((B * S, D), x.dtype),
            scratch_shapes=[
                pltpu.VMEM((B * S, D), bf16), pltpu.VMEM((FM, D), bf16), pltpu.VMEM((FM, D), bf16),
                pltpu.VMEM((128, D), bf16), pltpu.VMEM((FM + 128, D), bf16), pltpu.VMEM((B * S, D), bf16),
                pltpu.SemaphoreType.DMA((2 * len(fchunks) + 5,)), pltpu.SemaphoreType.DMA((nm,)),
            ],
            compiler_params=pltpu.CompilerParams(vmem_limit_bytes=100 * 2**20),
        )(x2, w_gate.T, w_up.T, w_down)
        return out.reshape(B, S, D)
    return fn

pallas_standalone__glu_gated_bilinear__prompt_kernel = jax.jit(make(512))
```

```python
import functools, itertools
import numpy as np
import jax
import jax.numpy as jnp
from jax import lax
import jax.experimental.pallas as pl
import jax.experimental.pallas.tpu as pltpu

f32 = jnp.float32
bf16 = jnp.bfloat16
u32 = jnp.uint32
NT = (((1,), (1,)), ((), ()))
T = 128

def dnt(a, b): return lax.dot_general(a, b, NT, preferred_element_type=f32)
def dnn(a, b): return jnp.dot(a, b, preferred_element_type=f32)
def as_bf16(v): return pltpu.bitcast(v, bf16)
def as_u32(v): return pltpu.bitcast(v, u32)
def ssum(terms):
    k = next((n for n, (s, _) in enumerate(terms) if s > 0), None)
    if k is None: return -ssum([(1, v) for _, v in terms])
    acc = terms[k][1] - ssum([(1, v) for _, v in terms[:k]]) if k else terms[0][1]
    for s, v in terms[k + 1:]: acc = acc + v if s > 0 else acc - v
    return acc
def combine(terms):
    un = lambda v, i: pltpu.unpack_elementwise(as_u32(v), index=i, packed_dtype=bf16, unpacked_dtype=f32)
    return pltpu.pack_elementwise([ssum([(s, un(v, i)) for s, v in terms]) for i in range(2)], packed_dtype=bf16)

def pairing(lab0, lab1, order="kind"):
    n0 = len(lab0); lab = list(lab0) + list(lab1); n = len(lab)
    edges = [(i, j) for i in range(n0) for j in range(n0, n) if lab[i] != lab[j]]
    nb = {c: [i + j - c for i, j in edges if c in (i, j)] for c in range(n)}
    Dw, Dv, G, V0, V1, Z = [], [], [], [], [], []
    for c in range(n):
        l = lab[c]; m = 1 if c < n0 else 0; q = 1 if c < n0 else -1
        Dw.append(([(1, (m, l))], [(1, (l, c))] + [(1, (lab[o], c)) for o in nb[c]], [(-q, (0, c)), (q, (1, c))]))
        Dv.append(([(1, (0, l)), (1, (1, l))], [(1, (l, c))] + [(-1, (l, o)) for o in nb[c]], [(1, (1 - m, c))]))
        for k in range(5):
            if k != l and k not in [lab[o] for o in nb[c]]:
                G += [([(1, (m_, k))], [(1, (k, c))], [(1, (m_, c))]) for m_ in range(2)]
    for i, j in edges:
        a, b = lab[i], lab[j]; lo, hi = sorted((a, b)); s = 1 if a < b else -1
        V0.append(([(1, (0, lo)), (-1, (0, hi))], [(1, (a, j))], [(s, (0, i)), (s, (0, j))]))
        V1.append(([(1, (1, lo)), (-1, (1, hi))], [(1, (b, i))], [(-s, (1, i)), (-s, (1, j))]))
        Z.append(([(1, (0, b)), (1, (1, a))], [(1, (a, j)), (1, (b, i))], [(1, (0, i)), (1, (1, j))]))
    if order == "kind": return Dw + G + V0 + V1 + Z + Dv
    if order == "pair":
        key = lambda p: tuple(i for _, i in p[0])
        return sorted(V0 + V1, key=lambda p: (p[0][0][1][1], p[0][1][1][1], p[0][0][1][0])) + Z + sorted(Dv, key=key) + Dw + G

class Multi:
    def __init__(self, cps): self.cps = cps
    def start(self):
        for c in self.cps: c.start()
    def wait(self):
        for c in self.cps: c.wait()

def make(nfirst=2, nloop=2, split0=3, only=None, mid_dma=True, flags=None):
    full = pairing(range(5), range(5))
    groups = [(pairing([0, 1, 2, 3], [4, 3, 2]), [10, 11, 12, 26, 23, 24, 25]),
              (full, [0, 1, 2, 3, 4, 13, 14, 15, 16, 17]),
              (full, [5, 6, 7, 8, 9, 18, 19, 20, 21, 22])]
    s2a = pairing(range(5), range(5), "pair")
    S7 = [([(1, (0, 0)), (1, (1, 1))], [(1, (0, 0)), (1, (1, 1))], [(1, (0, 0)), (1, (1, 1))]),
          ([(1, (1, 0)), (1, (1, 1))], [(1, (0, 0))], [(1, (1, 0)), (-1, (1, 1))]),
          ([(1, (0, 0))], [(1, (0, 1)), (-1, (1, 1))], [(1, (0, 1)), (1, (1, 1))]),
          ([(1, (1, 1))], [(1, (1, 0)), (-1, (0, 0))], [(1, (0, 0)), (1, (1, 0))]),
          ([(1, (0, 0)), (1, (0, 1))], [(1, (1, 1))], [(-1, (0, 0)), (1, (0, 1))]),
          ([(1, (1, 0)), (-1, (0, 0))], [(1, (0, 0)), (1, (0, 1))], [(1, (1, 1))]),
          ([(1, (0, 1)), (-1, (1, 1))], [(1, (1, 0)), (1, (1, 1))], [(1, (0, 0))])]
    P1 = [[(a, [(s, (k, cols[c])) for s, (k, c) in b], [(s, (m, cols[c])) for s, (m, c) in o]) for a, b, o in prods] for prods, cols in groups]
    P2 = [(o, [(s, (c, l)) for s, (l, c) in b], a) for a, b, o in s2a]
    for n0 in (0, 2):
        for a, b, o in S7:
            for k0 in (10, 12):
                P2.append(([(s, (m, k0 + k)) for s, (m, k) in a], [(s, (k0 + k, n0 + n)) for s, (k, n) in b], [(s, (m, n0 + n)) for s, (m, n) in o]))
    P2 += [([(1, (m, k))], [(1, (k, 4))], [(1, (m, 4))]) for m in range(2) for k in range(10, 14)]
    def norm(p):
        a, b, o = p
        if a[0][0] < 0: a = [(-s, i) for s, i in a]; o = [(-s, i) for s, i in o]
        return a, b, o
    P2 = [norm(p) for p in P2]
    slot = {}
    for tag, prods in [((1, g), P1[g]) for g in range(3)] + [((2, 0), P2)]:
        for r, (a, b, o) in enumerate(prods):
            if len(b) > 1: slot[tag, r] = len(slot)

    def kern(x_hbm, wg_hbm, wu_hbm, wd_hbm, o_hbm, x_v, wg_v, wu_v, wt_v, wd_v, o_v, wc_ref, sem, sem_o):
        S, D = x_hbm.shape
        F = wd_hbm.shape[0]
        FM = F // T * T; FT = F - FM
        ns = S // (2 * T)
        k_ = iter(range(64))
        def cp(src, dst, r0, n, d0=None): return pltpu.make_async_copy(src.at[pl.ds(r0, n)], dst.at[pl.ds(r0 if d0 is None else d0, n)], sem.at[next(k_)])
        x0 = cp(x_hbm, x_v, 0, nfirst * 2 * T)
        wa = Multi([cp(wg_hbm, wg_v, 10 * T, 3 * T)])
        wb = Multi([cp(wu_hbm, wu_v, 10 * T, 3 * T), cp(wg_hbm, wt_v, FM, FT, 0), cp(wu_hbm, wt_v, FM, FT, FT)])
        wgrp = [Multi([cp(wg_hbm, wg_v, a * T, 5 * T), cp(wu_hbm, wu_v, a * T, 5 * T)]) for a in (0, 5)]
        dcp = cp(wd_hbm, wd_v, 0, F)
        xr = cp(x_hbm, x_v, nfirst * 2 * T, S - nfirst * 2 * T)
        for c in [x0, wa, wb] + wgrp + [dcp, xr]: c.start()
        wd_v[pl.ds(F, T - FT), :] = jnp.zeros((T - FT, D), bf16)

        def w1_tile(k, n):
            c = slice(k * T, (k + 1) * T)
            if n < 13: return wg_v[pl.ds(n * T, T), c]
            if n < 26: return wu_v[pl.ds((n - 13) * T, T), c]
            return wt_v[:, c]
        def w2_tile(k, n): return wd_v[pl.ds(k * T, T), n * T:(n + 1) * T]
        def rhs(tag, r, form, tile, cache):
            if len(form) == 1: return tile(*form[0][1])
            if cache is None: return as_bf16(wc_ref[slot[tag, r]])
            if r not in cache:
                cache[r] = combine([(s, tile(*i)) for s, i in form])
                wc_ref[slot[tag, r]] = cache[r]
            return as_bf16(cache[r])
        class Lhs:
            def __init__(self, get): self.get = get; self.memo = {}
            def __call__(self, form):
                key = tuple(sorted(form, key=lambda t: t[1]))
                if key not in self.memo:
                    self.memo[key] = self.get(*form[0][1]).astype(bf16) if len(form) == 1 else ssum([(s, self.get(*i).astype(f32)) for s, i in form]).astype(bf16)
                return self.memo[key]
        class Acc:
            def __init__(self): self.terms = {}; self.last = None
            def add(self, form, p):
                key = [i for _, i in form]
                if self.last is not None and self.last[0] == key:
                    same = form[0][0] == self.last[1][0][0]
                    self.last = (key, self.last[1], self.last[2] + p if same else self.last[2] - p)
                else:
                    self.flush(); self.last = (key, form, p)
            def flush(self):
                if self.last is not None:
                    for s, i in self.last[1]: self.terms.setdefault(i, []).append((s, self.last[2]))
                self.last = None
            def result(self, i):
                self.flush()
                return ssum(self.terms[i])
        def x_lhs(r0): return Lhs(lambda m, k: x_v[pl.ds(r0 + m * T, T), k * T:(k + 1) * T])
        def stage1(g, idx, lhss, accs, cache):
            for r in idx:
                a, b, o = P1[g][r]
                w = rhs((1, g), r, b, w1_tile, cache)
                for L, acc in zip(lhss, accs): acc.add(o, dnt(L(a), w))
        def gate(g, acc, h):
            for n in groups[g][1]:
                for m in range(2):
                    if n < 13: h[m, n] = acc.result((m, n)) * acc.result((m, n + 13))
                    elif n == 26:
                        t = acc.result((m, n))
                        t = t * pltpu.roll(t, FT, 1)
                        h[m, 13] = jnp.where(lax.broadcasted_iota(jnp.int32, t.shape, 1) < FT, t, 0.0)
        def stage2(r0s, hs, cache):
            lhss = [Lhs(lambda m, k, h=h: h[m, k]) for h in hs]; accs = [Acc() for _ in hs]
            for r, (a, b, o) in enumerate(P2):
                w = rhs((2, 0), r, b, w2_tile, cache)
                for L, acc in zip(lhss, accs): acc.add(o, dnn(L(a), w))
            for r0, acc in zip(r0s, accs):
                for m in range(2):
                    for n in range(5): o_v[pl.ds(r0 + m * T, T), n * T:(n + 1) * T] = acc.result((m, n)).astype(bf16)
        def out_cp(i):
            r = pl.ds(pl.multiple_of(i * 2 * T, 2 * T), 2 * T)
            return pltpu.make_async_copy(o_v.at[r], o_hbm.at[r], sem_o.at[i])

        sel = lambda n: only is None or n in only
        x0.wait()
        r0s = [i * 2 * T for i in range(nfirst)]
        lhss = [x_lhs(r0) for r0 in r0s]; hs = [{} for _ in r0s]
        accs = [Acc() for _ in r0s]; cache = {}
        early = [r for r, (a, b, o) in enumerate(P1[0]) if all(n in (10, 11, 12) for _, (k, n) in b)] if split0 else []
        wa.wait()
        if sel("g2"): stage1(0, early, lhss, accs, cache)
        wb.wait()
        if sel("g2"):
            stage1(0, [r for r in range(len(P1[0])) if r not in early], lhss, accs, cache)
            for acc, h in zip(accs, hs): gate(0, acc, h)
        for g in (1, 2):
            wgrp[g - 1].wait()
            if sel("g2"):
                accs = [Acc() for _ in r0s]
                stage1(g, range(len(P1[g])), lhss, accs, {})
                for acc, h in zip(accs, hs): gate(g, acc, h)
        dcp.wait(); xr.wait()
        if sel("g2"): stage2(r0s, hs, {})
        for i in range(nfirst): out_cp(i).start()

        def body(it, carry):
            for s in range(nloop):
                i = nfirst + it * nloop + s
                r0 = pl.multiple_of(i * 2 * T, 2 * T)
                L = x_lhs(r0); h = {}
                for g in range(3):
                    acc = Acc()
                    stage1(g, range(len(P1[g])), [L], [acc], None)
                    gate(g, acc, h)
                stage2([r0], [h], None)
                if mid_dma: out_cp(i).start()
            if not mid_dma:
                for s in range(nloop): out_cp(nfirst + it * nloop + s).start()
            return carry
        if sel("loop"): lax.fori_loop(0, (ns - nfirst) // nloop, body, 0)
        else:
            for i in range(nfirst, ns): out_cp(i).start()
        for i in range(ns): out_cp(i).wait()

    def fn(x, w_gate, w_up, w_down):
        Bn, S, D = x.shape
        F = w_gate.shape[1]
        FM = F // T * T
        V = pltpu.VMEM
        out = pl.pallas_call(
            kern,
            in_specs=[pl.BlockSpec(memory_space=pl.ANY)] * 4,
            out_specs=pl.BlockSpec(memory_space=pl.ANY),
            out_shape=jax.ShapeDtypeStruct((Bn * S, D), x.dtype),
            scratch_shapes=[
                V((Bn * S, D), bf16), V((FM, D), bf16), V((FM, D), bf16), V((T, D), bf16), V((FM + T, D), bf16), V((Bn * S, D), bf16),
                V((len(slot), T // 2, T), u32),
                pltpu.SemaphoreType.DMA((12,)), pltpu.SemaphoreType.DMA((Bn * S // (2 * T),)),
            ],
            compiler_params=pltpu.CompilerParams(vmem_limit_bytes=100 * 2**20, flags=flags),
        )(x.reshape(Bn * S, D), w_gate.T, w_up.T, w_down)
        return out.reshape(Bn, S, D)
    return fn

pallas_standalone__glu_gated_bilinear__prompt_kernel = jax.jit(make(nloop=3))
```

```python
import functools, itertools
import numpy as np
import jax
import jax.numpy as jnp
from jax import lax
import jax.experimental.pallas as pl
import jax.experimental.pallas.tpu as pltpu

f32 = jnp.float32
bf16 = jnp.bfloat16
u32 = jnp.uint32
NT = (((1,), (1,)), ((), ()))
T = 128

def dnt(a, b): return lax.dot_general(a, b, NT, preferred_element_type=f32)
def dnn(a, b): return jnp.dot(a, b, preferred_element_type=f32)
def as_bf16(v): return pltpu.bitcast(v, bf16)
def as_u32(v): return pltpu.bitcast(v, u32)
def ssum(terms):
    k = next((n for n, (s, _) in enumerate(terms) if s > 0), None)
    if k is None: return -ssum([(1, v) for _, v in terms])
    acc = terms[k][1] - ssum([(1, v) for _, v in terms[:k]]) if k else terms[0][1]
    for s, v in terms[k + 1:]: acc = acc + v if s > 0 else acc - v
    return acc
def combine(terms):
    un = lambda v, i: pltpu.unpack_elementwise(as_u32(v), index=i, packed_dtype=bf16, unpacked_dtype=f32)
    return pltpu.pack_elementwise([ssum([(s, un(v, i)) for s, v in terms]) for i in range(2)], packed_dtype=bf16)

U, V, W = (1, 0), (0, 1), (1, 1)
METHOD = {"A": (W, V), "B": (W, U), "C": (U, V)}
def pairing(lab, cls):
    det = lambda x, y: x[0] * y[1] - x[1] * y[0]
    row = lambda c, d, s=1: [(s * d[m], (m, lab[c])) for m in range(2) if d[m]]
    col = lambda c, t, s=1: [(s * q, (m, c)) for m, q in enumerate((t[1], -t[0])) if q]
    n = len(lab)
    edges = []
    for a, b in itertools.combinations(range(5), 2):
        ca, cb = ([c for c in range(n) if lab[c] == l] for l in (a, b))
        if len(ca) > len(cb): ca, cb = cb, ca
        opts = [[(i, j) for i, j in zip(ca, p) if cls[i] != cls[j]] for p in itertools.permutations(cb, len(ca))]
        edges += min(opts, key=lambda o: (-len(o), sum("C" in (cls[i], cls[j]) for i, j in o)))
    coef = {(c, d): [(sg * det(*METHOD[cls[c]]), (lab[c], c))] for c in range(n) for d, sg in zip(METHOD[cls[c]], (1, -1))}
    out = []
    for i, j in sorted(tuple(sorted(e, key=lambda c: cls[c])) for e in edges):
        (w, v, u), = [(x, y, z) for x, y in (METHOD[cls[i]], METHOD[cls[i]][::-1]) for x2, z in (METHOD[cls[j]], METHOD[cls[j]][::-1]) if x == x2]
        s = det(u, v); x = det(w, v) * s; y = det(u, w) * s
        cij, cji = (lab[i], j), (lab[j], i)
        out.append(("V0", row(i, u) + row(j, u, -1), [(s, cij)], col(i, v) + col(j, v)))
        out.append(("V1", row(i, v) + row(j, v, -1), [(s, cji)], col(i, u) + col(j, u)))
        out.append(("Z", row(i, v) + row(j, u, x * y), [(s * x * y, cij), (s * x * y, cji)], col(i, v) + col(j, u, -x * y)))
        coef[i, w].append((-s * x, cij)); coef[i, v].append((-s * x, cji))
        coef[j, u].append((s * y, cij)); coef[j, w].append((s * y, cji))
    for c in range(n):
        m0, m1 = METHOD[cls[c]]
        out.append(("Dv", row(c, m0), coef[c, m0], col(c, m1)))
        out.append(("Dw", row(c, m1), coef[c, m1], col(c, m0)))
        for k in range(5):
            if k != lab[c] and not any(c in e and lab[e[0] + e[1] - c] == k for e in edges):
                out += [("G", [(1, (m, k))], [(1, (k, c))], [(1, (m, c))]) for m in range(2)]
    return out
def normal(a, b, o):
    a = sorted(a, key=lambda t: t[1]); o = sorted(o, key=lambda t: t[1])
    sa = a[0][0]; sb = max(s for s, _ in b)
    return [(s * sa, i) for s, i in a], [(s * sb, i) for s, i in b], [(s * sa * sb, i) for s, i in o]

class Multi:
    def __init__(self, cps): self.cps = cps
    def start(self):
        for c in self.cps: c.start()
    def wait(self):
        for c in self.cps: c.wait()

def plan(o1, o2, cls2):
    groups = [([0, 1, 2, 3, 4, 3, 2], "AAAABBB", [10, 11, 12, 26, 23, 24, 25]),
              (list(range(5)) * 2, "A" * 5 + "B" * 5, [0, 1, 2, 3, 4, 13, 14, 15, 16, 17]),
              (list(range(5)) * 2, "A" * 5 + "B" * 5, [5, 6, 7, 8, 9, 18, 19, 20, 21, 22])]
    P1 = []
    for lab, cls, cols in groups:
        prods = sorted(pairing(lab, cls), key=lambda p: o1.index(p[0]))
        P1.append([normal(a, [(s, (k, cols[c])) for s, (k, c) in b], [(s, (m, cols[c])) for s, (m, c) in o]) for _, a, b, o in prods])
    lab2 = list(range(5)) * 2 + [0, 1, 2, 3]
    prods = [(kd,) + normal(o, [(s, (c, l)) for s, (l, c) in b], a) for kd, a, b, o in pairing(lab2, cls2)]
    okey = lambda p: [i for _, i in p[3]]
    if o2 == "label": prods.sort(key=lambda p: (min(n for _, (_, n) in p[3]), max(n for _, (_, n) in p[3]) * (1 if p[0][0] in "VZ" else 9), p[0], okey(p)))
    elif o2 == "label2": prods.sort(key=lambda p: (min(n for _, (_, n) in p[3]), p[0][0] not in "VZ", p[0][0], okey(p)))
    else: prods.sort(key=lambda p: (o2.index(p[0][0]), okey(p)))
    return groups, P1, [p[1:] for p in prods]

def make(nfirst=2, nloop=2, feeds=((10, 11), (23, 24), (12, 25, 26), (0, 1, 2, 3, 4, 13, 14, 15, 16, 17), (5, 6, 7, 8, 9, 18, 19, 20, 21, 22)), o2f='heavylast', lag1=0, lag2=0, only=None, flags=None, o1=("G", "V0", "Dw", "V1", "Z", "Dv"), o2="label2", cls2="AAAAABBBBBCACB", pieces=((0, 3), (3, 1), (4, 1)), scopes=False, s2first='mix'):
    groups, P1, P2 = plan(o1, o2, cls2)
    slot = {}
    for tag, prods in [((1, g), P1[g]) for g in range(3)] + [((2, 0), P2)]:
        for r in range(len(prods)): slot[tag, r] = len(slot)

    def kern(x_hbm, wg_hbm, wu_hbm, wd_hbm, o_hbm, x_v, wg_v, wu_v, wt_v, wd_v, o_v, wc_ref, sem, sem_o):
        S, D = x_hbm.shape
        F = wd_hbm.shape[0]
        FM = F // T * T; FT = F - FM
        ns = S // (2 * T)
        k_ = iter(range(64))
        def cp(src, dst, r0, n, d0=None): return pltpu.make_async_copy(src.at[pl.ds(r0, n)], dst.at[pl.ds(r0 if d0 is None else d0, n)], sem.at[next(k_)])
        x0 = cp(x_hbm, x_v, 0, nfirst * 2 * T)
        def tiles_cp(ns_):
            out = []
            for src, dst, base in ((wg_hbm, wg_v, 0), (wu_hbm, wu_v, 13)):
                t = sorted(n - base for n in ns_ if base <= n < base + 13)
                for _, run in itertools.groupby(enumerate(t), lambda e: e[1] - e[0]):
                    run = [v for _, v in run]
                    out.append(cp(src, dst, run[0] * T, len(run) * T))
            if 26 in ns_: out += [cp(wg_hbm, wt_v, FM, FT, 0), cp(wu_hbm, wt_v, FM, FT, FT)]
            return Multi(out)
        wcp = [tiles_cp(f) for f in feeds]
        dcp = cp(wd_hbm, wd_v, 0, F)
        xr = cp(x_hbm, x_v, nfirst * 2 * T, S - nfirst * 2 * T)
        for c in [x0] + wcp + [dcp, xr]: c.start()
        wd_v[pl.ds(F, T - FT), :] = jnp.zeros((T - FT, D), bf16)

        def w1_tile(k, n):
            c = slice(k * T, (k + 1) * T)
            if n < 13: return wg_v[pl.ds(n * T, T), c]
            if n < 26: return wu_v[pl.ds((n - 13) * T, T), c]
            return wt_v[:, c]
        def w2_tile(k, n): return wd_v[pl.ds(k * T, T), n * T:(n + 1) * T]
        def rhs(tag, r, form, tile, first):
            if not first: return as_bf16(wc_ref[slot[tag, r]])
            v = combine([(s, tile(*i)) for s, i in form]) if len(form) > 1 else as_u32(tile(*form[0][1]))
            wc_ref[slot[tag, r]] = v
            return as_bf16(v)
        class Lhs:
            def __init__(self, get): self.get = get; self.memo = {}
            def __call__(self, form):
                key = tuple(form)
                if key not in self.memo:
                    self.memo[key] = self.get(*form[0][1]).astype(bf16) if len(form) == 1 else ssum([(s, self.get(*i).astype(f32)) for s, i in form]).astype(bf16)
                return self.memo[key]
        class Acc:
            def __init__(self): self.terms = {}; self.last = None
            def add(self, form, p):
                if self.last is not None and self.last[0] == form: self.last = (form, self.last[1] + p)
                elif self.last is not None and self.last[0] == [(-s, i) for s, i in form]: self.last = (self.last[0], self.last[1] - p)
                else:
                    self.flush(); self.last = (form, p)
            def flush(self):
                if self.last is not None:
                    for s, i in self.last[0]: self.terms.setdefault(i, []).append((s, self.last[1]))
                self.last = None
            def result(self, i):
                self.flush()
                return ssum(self.terms[i])
        def x_lhs(r0): return Lhs(lambda m, k: x_v[pl.ds(r0 + m * T, T), k * T:(k + 1) * T])
        def run(prods, tag, idx, tile, dot, lhss, accs, first, lag):
            idx = list(idx); n = len(idx) - lag; ws = {}
            for r in idx[:n]:
                a, b, o = prods[r]
                w = rhs(tag, r, b, tile, first)
                for L, acc in zip(lhss, accs): acc.add(o, dot(L(a), w))
            for L, acc in zip(lhss, accs):
                for r in idx[n:]:
                    a, b, o = prods[r]
                    if r not in ws: ws[r] = rhs(tag, r, b, tile, first)
                    acc.add(o, dot(L(a), ws[r]))
        def stage1(g, idx, lhss, accs, first, lag=0):
            run(P1[g], (1, g), idx, w1_tile, dnt, lhss, accs, first, lag)
        def gate(g, acc, h, late=None):
            for n in groups[g][2]:
                for m in range(2):
                    if n < 13: h[m, n] = acc.result((m, n)) * acc.result((m, n + 13))
                    elif n == 26:
                        def fin(t=acc.result((m, n)), m=m, h=h):
                            t = t * pltpu.roll(t, FT, 1)
                            h[m, 13] = jnp.where(lax.broadcasted_iota(jnp.int32, t.shape, 1) < FT, t, 0.0)
                        if late is None: fin()
                        else: late.append(fin)
        def out_cp(i, j):
            r = pl.ds(pl.multiple_of(i * 2 * T, 2 * T), 2 * T); c = pl.ds(pieces[j][0] * T, pieces[j][1] * T)
            return pltpu.make_async_copy(o_v.at[r, c], o_hbm.at[r, c], sem_o.at[i])
        def stage2(ids, hs, first):
            lhss = [Lhs(lambda m, k, h=h: h[m, k]) for h in hs]; accs = [Acc() for _ in hs]
            order = list(range(len(P2)))
            if first and o2f == "even": order = even(P2, order)
            elif first and o2f == "heavylast": order.sort(key=lambda r: len(P2[r][1]) > 2)
            elif first and o2f == "heavyfirst": order.sort(key=lambda r: len(P2[r][1]) <= 2)
            run(P2, (2, 0), order, w2_tile, dnn, lhss, accs, first, lag2 if first else 0)
            for i, acc in zip(ids, accs):
                for j, (n0, nn) in enumerate(pieces):
                    for n in range(n0, n0 + nn):
                        for m in range(2): o_v[pl.ds(pl.multiple_of(i * 2 * T + m * T, T), T), n * T:(n + 1) * T] = acc.result((m, n)).astype(bf16)
                    out_cp(i, j).start()

        def even(prods, idx):
            idx = list(idx)
            heavy = [r for r in idx if len(prods[r][1]) > 2]; light = [r for r in idx if r not in heavy]
            keyed = [((n + 0.5) / len(l), r) for l in (heavy, light) for n, r in enumerate(l)]
            return [r for _, r in sorted(keyed)]
        sel = lambda n: only is None or n in only
        import contextlib
        scope = (lambda n: jax.named_scope(n)) if scopes else (lambda n: contextlib.nullcontext())
        x0.wait()
        lhss = [x_lhs(i * 2 * T) for i in range(nfirst)]; hs = [{} for _ in lhss]
        accs = [[Acc() for _ in lhss] for _ in P1]
        todo = [list(range(len(p))) for p in P1]; have = set(); pending = []
        for bi, (f, c) in enumerate(zip(feeds, wcp)):
            c.wait(); have |= set(f)
            with scope(f"b{bi}"):
                while pending: pending.pop(0)()
                for g in range(3):
                    now = [r for r in todo[g] if all(n in have for _, (k, n) in P1[g][r][1])]
                    if len(now) < len(todo[g]): now = now[:len(now) // 2 * 2]
                    if not now: continue
                    todo[g] = [r for r in todo[g] if r not in now]
                    if sel("g2"):
                        stage1(g, even(P1[g], now), lhss, accs[g], True, 0 if todo[g] else lag1)
                        if not todo[g]:
                            for acc, h in zip(accs[g], hs): gate(g, acc, h, pending)
        dcp.wait()
        with scope("s2"):
          if sel("g2"):
            if s2first == "seq":
                for i in range(nfirst): stage2([i], [hs[i]], i == 0)
            else: stage2(range(nfirst), hs, True)
          else: pl.delay(10)

        def body(it, carry):
            for s in range(nloop):
                i = nfirst + it * nloop + s
                L = x_lhs(pl.multiple_of(i * 2 * T, 2 * T)); h = {}
                for g in range(3):
                    acc = Acc()
                    stage1(g, range(len(P1[g])), [L], [acc], False)
                    gate(g, acc, h)
                stage2([i], [h], False)
            return carry
        xr.wait()
        with scope("loop"):
            if sel("loop"): lax.fori_loop(0, (ns - nfirst) // nloop, body, 0)
        for i in range(ns):
            if sel("g2" if i < nfirst else "loop"):
                for j in range(len(pieces)): out_cp(i, j).wait()

    def fn(x, w_gate, w_up, w_down):
        Bn, S, D = x.shape
        F = w_gate.shape[1]
        FM = F // T * T
        M = pltpu.VMEM
        out = pl.pallas_call(
            kern,
            in_specs=[pl.BlockSpec(memory_space=pl.ANY)] * 4,
            out_specs=pl.BlockSpec(memory_space=pl.ANY),
            out_shape=jax.ShapeDtypeStruct((Bn * S, D), x.dtype),
            scratch_shapes=[
                M((Bn * S, D), bf16), M((FM, D), bf16), M((FM, D), bf16), M((T, D), bf16), M((FM + T, D), bf16), M((Bn * S, D), bf16),
                M((len(slot), T // 2, T), u32),
                pltpu.SemaphoreType.DMA((24,)), pltpu.SemaphoreType.DMA((Bn * S // (2 * T),)),
            ],
            compiler_params=pltpu.CompilerParams(vmem_limit_bytes=100 * 2**20, flags=flags),
        )(x.reshape(Bn * S, D), w_gate.T, w_up.T, w_down)
        return out.reshape(Bn, S, D)
    return fn

pallas_standalone__glu_gated_bilinear__prompt_kernel = jax.jit(make(nloop=3))
```

```python
import functools
import itertools

import numpy as np
import jax
import jax.numpy as jnp
from jax import lax
import jax.experimental.pallas as pl
import jax.experimental.pallas.tpu as pltpu

f32, bf16, u32 = jnp.float32, jnp.bfloat16, jnp.uint32
T = 128
H = T // 2
FIRST = 2
UNROLL = 3


def vectors(text):
    return np.array([["-0+".index(c) - 1 for c in word] for word in text.split()])


NINE = dict(
    R=vectors("0000- 00+0+ 00+00 -0000 +-000 0-000 -000- +-+0+ 0-+00 0+00+ 0+000 000+0 00--0 00-00 000+- 0+--+ 0+-00 "
              "000+0 -0000 00+-0 -00+- 0-0+0 ++000 -00+- +0-00 -00+0"),
    B=vectors("00000+000 0-000-000 0-0000000 000+0-000 00--0+000 00-000000 000+00000 0---00000 0--000000 0000--000 "
              "0000-0000 00000-0-0 00000+0++ 00000000+ 0000000-0 0000-00++ 0000-000+ +00000000 000000+00 --0000000 "
              "+00+00000 +0+000000 0000-0+00 000000+-0 000000-0+ -00000+00"),
    cls="CBABACACBABABCBCABACCACCBC",
    lines=((2, 1, 0), (4, 3, 5), (6, 3, 0), (4, 1, 7), (2, 8, 5), (6, 8, 7), (9, 10, 0), (11, 12, 13), (11, 14, 0),
           (9, 12, 15), (16, 10, 13), (16, 14, 15), (2, 17, 19), (6, 17, 20), (21, 17, 5), (18, 10, 22), (18, 14, 23),
           (18, 24, 13), (18, 17, 25)))
SIX = dict(
    R=vectors("000-0 +000+ +00-+ 00++0 00-0- 000+- 00+00 +0-00 +0000 0+000 -0000 -+000 0+0-0 0000+ 0+0-+ -++00 +--00"),
    B=vectors("00000+ 00-000 00-00+ 000+0- 00+0+0 00+++- 000+00 0000+0 000++0 0-0000 +00000 +-0000 0-000+ +0-000 "
              "+--00+ +-0-00 0-00+0"),
    cls="BACACBCBACBAACBBA",
    lines=((0, 1, 2), (5, 3, 4), (0, 3, 6), (7, 1, 4), (5, 8, 2), (7, 8, 6), (10, 11, 9), (0, 12, 9), (10, 1, 13),
           (14, 11, 2), (14, 12, 13), (15, 11, 6), (7, 16, 9)))
DOWN = dict(
    R=vectors("-0+00 ++000 0++00 000+0 0-000 0-0+0 -0++0 +0000 00++0 00-00 0000+ 00-0+ -0000 ++00+ 0+00+"),
    B=(vectors("+00000 00000+ +0000+ 00+000 00-0+0 0000+0 +0+000 00-0++ +000++ 0-0000 000+00 0-0+00 +-0000 000+0+ +-0+0+"),
       vectors("0-0000 000-00 0-0-00 0+00+0 00000- 0+00+- 0000+0 000-0- 000-+- +00000 00+000 +0+000 +-0000 00+-00 +-+-00")),
    cls="CABABCBCAABCBCA",
    lines=((1, 2, 0), (3, 4, 5), (3, 6, 0), (1, 4, 7), (8, 2, 5), (8, 6, 7), (9, 10, 11), (9, 12, 0), (1, 10, 13),
           (14, 2, 11), (14, 12, 13)),
    single=(vectors("000++")[0], "A"),
    links=((27, 30, 1, -1), (5, 30, -1, 1), (11, 31, -1, 1), (25, 31, -1, 1), (19, 32, 1, 1), (21, 32, -1, -1), (3, 10, 1, 1)))

UP_DIRS = np.array([[1, 1], [-1, 1]])
DOWN_DIRS = np.array([[1, 0], [0, 1]])

NINE_TILES = (9, 22, 10, 23, 11, 12, 24, 26, 25)
SIX_TILES = (0, 1, 13, 2, 14, 15)

AHEAD = (64, 40, 65, 56, 42, 38, 17, 43, 35, 66, 8, 50, 57, 39, 15, 6, 14, 55, 53, 2, 41, 16, 11, 4, 51, 70, 47, 10, 34,
         9, 12, 45, 3, 63, 44, 52)
FIRST_NINE = ((128, 80, 130, 112, 84, 76, 34, 86, 70, 132, 16, 100, 114, 78, 30, 12, 28, 110, 106, 4, 82, 32, 22, 8),
              (87, 77, 35, 133, 85, 102, 71, 101, 29, 5, 17, 79, 111, 107, 115, 13, 83, 31, 129, 9, 113, 81, 131, 141,
              23, 140, 33, 103, 94, 20, 68, 69, 18, 24, 19, 25, 21, 95, 90, 91), (89, 6, 126, 7, 127, 88, 104, 105, 14,
              108, 0, 62, 1, 15, 109, 63, 26, 10, 27, 11, 64, 122, 65, 123, 60, 44, 61, 124, 45, 66, 67, 36, 40, 117,
              37, 41, 38, 39, 125, 116, 48, 42, 49, 43, 118, 50, 119, 51, 46, 120, 47, 121, 134, 58, 135, 59, 92, 136,
              93, 137, 72, 96, 73, 97, 138, 56, 139, 57, 74, 99, 98, 75, 54, 2, 55, 3), (52, 53))
FIRST_SIX = ((45, 88, 44, 89, 82, 58, 83, 59, 54, 56, 55, 57, 20, 21, 53, 60, 52, 84, 61, 85, 48, 62, 49, 63, 86, 42,
             87, 43, 90, 64, 91, 65, 66, 50, 67, 51, 46, 38, 39, 36, 80, 92, 81, 93, 47, 10, 37, 11, 16, 22, 17, 23, 30,
             12, 31, 13, 8, 70, 9, 71, 18, 74, 19, 75, 14, 76, 15, 77, 26, 4, 27, 5, 2, 68, 3, 69, 34, 6, 35, 7, 72, 28,
             73, 29, 32, 78, 33, 79, 24, 0, 25, 1, 40, 41), (88, 52, 89, 53, 54, 44, 55, 45, 84, 56, 85, 57, 60, 40, 61,
             41, 58, 62, 59, 63, 90, 86, 91, 87, 46, 80, 47, 81, 42, 48, 43, 49, 82, 50, 83, 51, 38, 8, 39, 9, 64, 66,
             65, 67, 22, 36, 23, 37, 76, 10, 77, 11, 92, 16, 93, 17, 14, 30, 15, 31, 20, 12, 21, 13, 70, 18, 71, 19, 74,
             68, 75, 69, 34, 26, 35, 27, 32, 28, 33, 29, 2, 6, 3, 7, 78, 24, 79, 25, 72, 0, 73, 1, 4, 5))
FIRST_DOWN = (149, 26, 4, 161, 27, 148, 5, 160, 0, 60, 1, 24, 61, 211, 210, 86, 87, 48, 166, 182, 157, 183, 108, 167,
              25, 49, 64, 156, 65, 84, 85, 109, 128, 192, 129, 193, 198, 112, 199, 177, 200, 176, 201, 89, 113, 54, 188,
              55, 189, 88, 28, 29, 110, 52, 111, 53, 196, 114, 197, 115, 68, 8, 69, 9, 194, 178, 195, 179, 50, 150, 51,
              151, 66, 173, 67, 172, 90, 130, 91, 131, 171, 63, 2, 184, 170, 174, 3, 185, 62, 30, 31, 175, 164, 186,
              165, 135, 134, 187, 11, 10, 180, 76, 181, 77, 20, 6, 21, 7, 81, 16, 23, 17, 80, 158, 22, 159, 70, 132, 71,
              116, 162, 145, 163, 133, 56, 117, 144, 57, 146, 82, 147, 83, 208, 33, 32, 209, 202, 18, 203, 78, 94, 19,
              95, 79, 92, 136, 93, 137, 96, 46, 97, 47, 104, 118, 105, 119, 190, 58, 191, 59, 204, 106, 169, 205, 107,
              168, 44, 45, 38, 152, 124, 153, 39, 121, 120, 125, 72, 12, 73, 13, 138, 98, 139, 99, 140, 14, 141, 41,
              154, 40, 155, 127, 212, 206, 213, 207, 37, 126, 143, 74, 15, 142, 34, 75, 123, 36, 102, 122, 100, 35, 101,
              103, 42, 43)
LOOP = (((39, 65, 38, 51, 40, 41, 64, 42, 70, 10, 50, 34, 4, 3, 52, 17, 43, 66, 35, 55, 2, 15, 57, 14, 56, 16, 5, 11, 9, 53,
         8, 6, 12, 7, 67, 54, 23, 18, 13, 62, 30, 32, 59, 22, 31, 33, 24, 45, 61, 60, 25, 63, 20, 44, 0, 58, 1, 21, 68, 19,
         48, 49, 46, 47, 36, 69, 37, 27, 29, 26, 28), (26, 46, 22, 31, 27, 21, 45, 23, 20, 19, 29, 32, 30, 25, 43, 40, 41,
         33, 24, 28, 44, 1, 42, 18, 35, 11, 4, 2, 37, 8, 17, 5, 15, 10, 34, 9, 12, 36, 38, 3, 7, 14, 13, 39, 16, 0, 6), (22,
         40, 26, 46, 27, 29, 43, 20, 19, 45, 28, 44, 31, 25, 15, 33, 30, 41, 24, 32, 1, 23, 42, 11, 18, 4, 8, 21, 10, 2, 6,
         36, 17, 34, 35, 38, 13, 37, 9, 16, 12, 0, 7, 5, 39, 3, 14), (26, 46, 22, 27, 21, 40, 29, 45, 30, 32, 17, 20, 19, 41,
         28, 24, 23, 44, 33, 31, 39, 25, 14, 11, 18, 16, 38, 4, 1, 42, 6, 2, 8, 43, 10, 35, 9, 34, 15, 5, 7, 13, 37, 3, 0,
         12, 36), (30, 13, 80, 2, 83, 0, 25, 12, 24, 14, 42, 43, 94, 105, 32, 91, 54, 26, 56, 74, 27, 88, 93, 85, 99, 64, 96,
         100, 92, 1, 33, 44, 55, 75, 78, 57, 89, 81, 31, 5, 97, 86, 15, 87, 65, 35, 4, 73, 28, 58, 66, 8, 72, 10, 38, 40, 67,
         90, 104, 101, 79, 41, 3, 82, 98, 45, 39, 34, 48, 9, 68, 11, 29, 59, 16, 46, 23, 52, 22, 102, 17, 18, 47, 69, 95, 77,
         62, 84, 53, 60, 49, 6, 36, 76, 19, 70, 61, 63, 106, 103, 37, 50, 20, 71, 7, 21, 51)),
        ((38, 39, 64, 40, 41, 50, 51, 70, 10, 42, 65, 4, 3, 17, 66, 55, 35, 52, 15, 14, 2, 5, 43, 11, 9, 57, 16, 56, 53, 8,
         6, 34, 12, 32, 7, 54, 18, 13, 62, 24, 67, 59, 33, 30, 61, 45, 25, 22, 23, 60, 28, 63, 20, 36, 44, 58, 19, 0, 1, 48,
         46, 21, 47, 49, 69, 37, 68, 27, 29, 26, 31), (5, 28, 46, 22, 26, 27, 24, 40, 45, 6, 30, 41, 32, 44, 33, 20, 1, 42,
         31, 19, 15, 25, 39, 18, 11, 4, 2, 8, 29, 13, 10, 9, 21, 38, 35, 43, 16, 34, 17, 37, 23, 14, 12, 36, 3, 0, 7), (30,
         26, 27, 45, 20, 40, 19, 22, 41, 28, 46, 1, 29, 21, 32, 23, 31, 25, 5, 33, 43, 44, 42, 11, 18, 4, 2, 34, 24, 10, 6,
         17, 16, 39, 15, 13, 37, 8, 35, 9, 0, 36, 38, 14, 12, 7, 3), (20, 18, 31, 33, 45, 40, 46, 34, 19, 44, 26, 41, 28, 21,
         35, 30, 32, 43, 23, 4, 24, 25, 2, 1, 42, 11, 22, 8, 29, 27, 17, 6, 5, 15, 10, 37, 38, 16, 13, 9, 36, 39, 14, 12, 3,
         0, 7), (30, 13, 83, 80, 0, 2, 12, 25, 24, 105, 43, 32, 42, 94, 91, 54, 26, 56, 74, 27, 88, 64, 1, 93, 96, 100, 99,
         92, 85, 14, 44, 55, 75, 78, 57, 89, 81, 31, 65, 97, 33, 86, 15, 87, 5, 35, 4, 34, 28, 58, 66, 72, 10, 38, 8, 40, 67,
         90, 104, 101, 79, 41, 3, 82, 98, 45, 39, 73, 48, 9, 68, 17, 11, 29, 59, 16, 46, 23, 52, 22, 102, 18, 69, 62, 49, 84,
         47, 95, 77, 53, 60, 6, 36, 76, 19, 70, 61, 63, 106, 103, 7, 37, 50, 20, 71, 21, 51)),
        ((65, 38, 39, 64, 40, 41, 70, 50, 3, 51, 42, 34, 4, 52, 17, 66, 43, 10, 35, 8, 55, 2, 14, 15, 57, 16, 9, 56, 5, 6,
         11, 54, 53, 7, 18, 12, 67, 13, 62, 32, 24, 45, 33, 20, 61, 22, 25, 59, 23, 60, 31, 63, 30, 44, 58, 19, 0, 1, 21, 36,
         68, 48, 46, 47, 49, 69, 37, 29, 27, 28, 26), (43, 26, 46, 22, 40, 27, 45, 30, 29, 20, 42, 17, 21, 23, 41, 28, 19,
         11, 18, 31, 38, 24, 44, 33, 1, 4, 2, 8, 6, 5, 32, 15, 10, 34, 35, 9, 13, 37, 36, 25, 16, 39, 14, 3, 0, 7, 12), (21,
         26, 46, 11, 40, 27, 45, 30, 20, 28, 29, 43, 25, 42, 18, 19, 32, 23, 31, 33, 24, 1, 22, 44, 41, 4, 2, 8, 17, 6, 5,
         35, 38, 10, 34, 15, 9, 14, 16, 13, 37, 36, 39, 12, 3, 0, 7), (40, 46, 45, 26, 27, 30, 20, 24, 29, 43, 21, 41, 22,
         32, 31, 28, 25, 19, 36, 23, 39, 44, 1, 33, 42, 11, 18, 4, 8, 17, 10, 5, 2, 15, 6, 34, 35, 9, 16, 0, 13, 37, 14, 12,
         3, 38, 7), (30, 13, 83, 0, 80, 2, 12, 25, 24, 43, 42, 94, 93, 105, 32, 91, 54, 26, 56, 27, 88, 74, 85, 99, 64, 96,
         100, 92, 1, 14, 44, 55, 75, 78, 57, 31, 81, 65, 97, 86, 89, 35, 4, 5, 33, 15, 87, 34, 28, 58, 66, 8, 72, 10, 38, 40,
         67, 90, 104, 79, 101, 41, 3, 82, 98, 45, 39, 73, 48, 9, 68, 18, 11, 29, 46, 52, 22, 59, 69, 16, 23, 102, 17, 62, 84,
         47, 95, 77, 49, 53, 60, 61, 76, 19, 6, 70, 36, 103, 7, 37, 63, 106, 50, 20, 71, 21, 51)),)

WHOLE = (((0, 2, 0, 5),),)
PIECES = (((0, 2, 0, 3),), ((0, 1, 3, 4),), ((1, 2, 3, 4), (0, 2, 4, 5)))


def scheme(R, B, cls, lines, dirs):
    du, dv = dirs
    pick = {"A": (du + dv, dv), "B": (du + dv, du), "C": (du, dv)}
    row = lambda r, d: np.outer(d, r)
    col = lambda b, d: np.outer((d[1], -d[0]), b)
    A, C = [], []
    for r, b, c in zip(R, B, cls):
        A += [row(r, pick[c][0]), row(r, pick[c][1])]
        C += [col(b, pick[c][1]), col(b, pick[c][0])]
    for line in lines:
        i, j, k = sorted(line, key=lambda p: cls[p])
        rel = lambda M: next(s for s in (1, -1) for q in (1, -1) if np.array_equal(M[i] + s * M[j], q * M[k]))
        A.append(row(R[i], dv) - rel(R) * row(R[j], du))
        C.append(col(B[i], dv) - rel(B) * col(B[j], du))
    A, C = np.array(A), np.array(C)
    p, n = A.shape[2], C.shape[2]
    M = np.einsum("rap,rbn->apbnr", A, C).reshape(-1, len(A))
    eye = [np.eye(s, dtype=int) for s in (2, p, n)]
    want = (du[0] * dv[1] - du[1] * dv[0]) * np.einsum("ab,pq,nm->apbnqm", *eye).reshape(-1, p * n)
    W = np.rint(np.linalg.solve((M.T @ M).astype(float), (M.T @ want).astype(float))).astype(int)
    assert np.array_equal(M @ W, want)
    return A, W.reshape(-1, p, n), C


def down_scheme():
    d = DOWN
    npt, nln = len(d["cls"]), len(d["lines"])
    R, B, cls, lines, twin = [], [], "", [], []
    for k in range(2):
        for half in range(2):
            b = np.zeros((npt, 27), int)
            b[:, 12 * k + half:12 * k + 12:2] = d["B"][k]
            lines += [tuple(len(R) + p for p in line) for line in d["lines"]]
            R += list(d["R"]); B += list(b); cls += d["cls"]
        twin += [(2 * k * npt + p, (2 * k + 1) * npt + p) for p in range(npt)]
    z = len(R)
    R += [d["single"][0]] * 3; B += list(np.eye(27, dtype=int)[24:]); cls += d["single"][1] * 3
    twin += [(z, z + 1), (z, z + 2), (z + 2, z + 1)]
    points = twin[:-2] + [(z + 2, None)]
    for i, j, mu, lam in d["links"]:
        points.append((len(R), len(R) + 1))
        for a, b in zip(twin[i], twin[j]):
            lines.append((a, b, len(R)))
            R.append(R[a] + mu * R[b]); B.append(B[a] + lam * B[b])
            cls += next(c for c in "ABC" if c not in (cls[a], cls[b]))
    A, W, C = scheme(np.array(R), np.array(B), cls, lines, DOWN_DIRS)
    n = 2 * len(R)
    pairs = [(2 * a + e, None if b is None else 2 * b + e) for a, b in points for e in range(2)]
    pairs += [(n + 2 * k * nln + t, n + (2 * k + 1) * nln + t) for k in range(2) for t in range(nln)]
    pairs += [(n + 4 * nln + 2 * t, n + 4 * nln + 2 * t + 1) for t in range(len(d["links"]))]
    assert sorted(p for e in pairs for p in e if p is not None) == list(range(len(A)))
    rows, halves, cols = [], [], []
    for a, b in pairs:
        lo = C[a]
        hi = lo[:, list(range(25)) + [26, 25]] if b is None else C[b]
        mixed = np.stack([lo[:, p] * hi[:, q].any() for p, q in ((24, 25), (24, 26), (26, 25))], 1)
        assert b is None or (np.array_equal(A[a], A[b]) and np.array_equal(lo[:, 0:24:2], hi[:, 1:24:2]))
        assert not lo[:, 1:26:2].any() and not hi[:, 0:26:2].any()
        assert np.array_equal(mixed @ [[1, 0], [1, 0], [0, 1]], lo[:, [24, 26]])
        assert np.array_equal(mixed @ [[1, 0], [0, 1], [1, 0]], hi[:, [25, 26]])
        rows.append(A[a])
        cols.append(np.concatenate([lo[:, 0:24:2], mixed], 1))
        halves += [W[a], 0 * W[a] if b is None else W[b]]
    return np.array(rows), np.array(halves), np.array(cols)


class Chain:
    def __init__(self, forms):
        forms = forms.reshape(len(forms), -1)
        n = self.n = forms.shape[1]

        def canon(v):
            s = 1 if v[np.flatnonzero(v)[0]] > 0 else -1
            return s, tuple((s * v).tolist())

        vec = list(np.eye(n, dtype=int))
        node = {tuple(v.tolist()): i for i, v in enumerate(vec)}
        todo = [k for k in dict.fromkeys(canon(f)[1] for f in forms) if k not in node]
        self.steps, reach, done = [], {}, 0
        while todo:
            for b in range(done, len(vec)):
                for a in range(b + 1):
                    for s in (1, -1):
                        v = vec[a] + s * vec[b]
                        if v.any():
                            sg, key = canon(v)
                            reach.setdefault(key, (sg, a, sg * s, b))
            done = len(vec)
            now = [t for t in todo if t in reach]
            if not now:
                score = {}
                for t in todo:
                    for v in vec:
                        for s in (1, -1):
                            h = canon(np.array(t) + s * v)[1]
                            if h in reach and h not in node:
                                score[h] = score.get(h, 0) + 1
                now = [max(score, key=score.get)]
            for t in now:
                node[t] = len(vec); vec.append(np.array(t)); self.steps.append(reach[t])
            todo = [t for t in todo if t not in node]
        self.where = [(canon(f)[0], node[canon(f)[1]]) for f in forms]


class Shared:
    def __init__(self, sums, uses=99):
        self.where, self.terms, self.kept, key = [], [], {}, {}
        for t in sums:
            t = sorted(t, key=lambda e: e[1])
            sg = t[0][0] if t else 1
            t = tuple((q * sg, i) for q, i in t)
            if t not in key:
                key[t] = len(self.terms); self.terms.append(list(t))
            self.where.append((sg, key[t]))
        while True:
            count = {}
            for t in self.terms:
                for (p, a), (q, b) in itertools.combinations(t, 2):
                    count[a, p * q, b] = count.get((a, p * q, b), 0) + 1
            a, s, b = best = max(count, key=count.get)
            if count[best] < uses:
                break
            new = (99, len(self.kept))
            self.kept[new] = [(1, a), (s, b)]
            for t in self.terms:
                for p in (1, -1):
                    if (p, a) in t and (p * s, b) in t:
                        t.remove((p, a)); t.remove((p * s, b)); t.append((p, new))
        used = set(tuple(t) for t in self.terms)
        for n, t in enumerate(self.terms):
            rest, part = list(t), []

            def name(e):
                z = sorted(part + list(e), key=lambda x: x[1])
                return tuple((q * z[0][0], i) for q, i in z)

            while rest:
                e = min(itertools.combinations(rest, 1 if part else min(2, len(rest))), key=lambda e: name(e) in used)
                used.add(name(e)); part += e; rest = [x for x in rest if x not in e]
            self.terms[n] = part


def along(forms, du, dv):
    split = lambda v: next((q, p) for q in (0, 1, -1) for p in (0, 1, -1) if np.array_equal(v, q * du + p * dv))
    return [[(s, (d, c)) for c in range(f.shape[1]) for d, s in enumerate(split(f[:, c])) if s] for f in forms]


def entries(forms):
    return [[(int(f[a, b]), (int(a), int(b))) for a, b in zip(*np.nonzero(f))] for f in forms]


def signed_sum(terms):
    s0, acc = terms[0]
    for s, v in terms[1:]:
        if s == s0:
            acc = acc + v
        elif s0 > 0:
            acc = acc - v
        else:
            s0, acc = 1, v - acc
    return s0, acc


def value(v):
    return v() if callable(v) else v


class Operands:
    def __init__(self, table, get, finish, once=None):
        self.table, self.get, self.finish, self.made, self.kept = table, get, finish, {}, {}
        self.once, self.seen = once, {}

    def total(self, terms):
        out = []
        for q, e in terms:
            if self.once and e not in self.table.kept and e not in self.seen:
                self.seen[e] = True
                s, v = self.once(*e)
            else:
                if e not in self.kept:
                    self.kept[e] = self.total(self.table.kept[e]) if e in self.table.kept else self.get(*e)
                s, v = self.kept[e]
            out.append((q * s, value(v)))
        return signed_sum(out)

    def __call__(self, r):
        s, i = self.table.where[r]
        if i not in self.made:
            q, v = self.total(self.table.terms[i])
            self.made[i] = (q, self.finish(v))
        return s * self.made[i][0], self.made[i][1]


class Results:
    def __init__(self, chain, done):
        self.chain, self.done, self.terms = chain, done, {}
        self.left = [0] * (chain.n + len(chain.steps))
        for i in [i for _, i in chain.where] + [i for _, a, _, b in chain.steps for i in (a, b)]:
            self.left[i] += 1

    def add(self, r, sign, p):
        s, i = self.chain.where[r]
        self.put(i, s * sign, p)

    def put(self, i, s, v):
        self.terms.setdefault(i, []).append((s, v))
        self.left[i] -= 1
        if self.left[i]:
            return
        s, v = signed_sum(self.terms.pop(i))
        if i < self.chain.n:
            return self.done(i, s, v)
        sa, a, sb, b = self.chain.steps[i - self.chain.n]
        self.put(a, sa * s, v)
        self.put(b, sb * s, v)


class Rows:
    def __init__(self, even, odd):
        self.even, self.odd = even, odd

    def __add__(self, o):
        return Rows(self.even + o.even, self.odd + o.odd)

    def __sub__(self, o):
        return Rows(self.even - o.even, self.odd - o.odd)

    def packed(self):
        return pltpu.pack_elementwise([self.even, self.odd], packed_dtype=bf16)

    @staticmethod
    def once(tile):
        words = pltpu.bitcast(tile, u32)
        return Rows(pltpu.bitcast(words << 16, f32), pltpu.bitcast(words & np.uint32(0xFFFF0000), f32))

    @staticmethod
    def of(tile):
        words = pltpu.bitcast(tile, u32)
        return Rows(*[pltpu.unpack_elementwise(words, index=i, packed_dtype=bf16, unpacked_dtype=f32) for i in range(2)])


@functools.cache
def plan():
    nine, six, down = scheme(**NINE, dirs=UP_DIRS), scheme(**SIX, dirs=UP_DIRS), down_scheme()
    x_sums = along(np.concatenate([nine[0], six[0]]), *UP_DIRS)
    h_sums = along(down[2], *[np.array([d[1], -d[0]]) for d in DOWN_DIRS])
    every = lambda order, pairs, part: sorted(order) == list(range(pairs * len(part[0])))
    assert every(sum(FIRST_NINE, ()), FIRST, nine) and all(every(o, FIRST, six) for o in FIRST_SIX) and every(FIRST_DOWN, FIRST, down)
    assert all(every(o, 1, part) for orders in LOOP for o, part in zip(orders, (nine, six, six, six, down), strict=True))
    return dict(needs=[np.nonzero(w)[1] for w in nine[1]],
                x=Shared(x_sums), h=Shared(h_sums), x_first=Shared(x_sums, 5), h_first=Shared(h_sums, 5),
                w_nine=Shared(entries(nine[1]), 5), w_six=Shared(entries(six[1]), 3), w_down=Shared(entries(down[1]), 4),
                nine=Chain(nine[2]), six=Chain(six[2]), out=Chain(down[0]))


def out_copy(o_v, o_hbm, sem, i, m0, m1, n0, n1):
    r, c = pl.ds(pl.multiple_of((i * 2 + m0) * T, T), (m1 - m0) * T), pl.ds(n0 * T, (n1 - n0) * T)
    return pltpu.make_async_copy(o_v.at[i, pl.ds(m0 * T, (m1 - m0) * T), c], o_hbm.at[r, c], sem.at[0])


def kernel(x_hbm, wg_hbm, wu_hbm, wd_hbm, o_hbm, o_v, sem_out, *scratch):
    pl.run_scoped(functools.partial(compute, x_hbm, wg_hbm, wu_hbm, wd_hbm, o_hbm, o_v, sem_out, *scratch),
                  pltpu.SemaphoreType.DMA((13,)))
    for i in range(x_hbm.shape[0] // (2 * T)):
        last = i >= FIRST and (i - FIRST) % UNROLL == UNROLL - 1
        for piece in sum(PIECES if last else WHOLE, ()):
            out_copy(o_v, o_hbm, sem_out, i, *piece).wait()


def compute(x_hbm, wg_hbm, wu_hbm, wd_hbm, o_hbm, o_v, sem_out,
            x_v, wg_v, wu_v, wd_v, xs_v, h_v, nine_v, six_v, down_v, sem):
    P = plan()
    S, F = x_hbm.shape[0], wd_hbm.shape[0]
    FM = F // T * T
    n9, n6 = len(P["nine"].where), len(P["six"].where)
    DOWN_PART = 4

    slots = itertools.count()

    def copy(src, dst, r0, r1):
        r = pl.ds(r0, min(r1, src.shape[0]) - r0)
        return pltpu.make_async_copy(src.at[r], dst.at[r], sem.at[next(slots)])

    gates, ups = [lambda t0, t1, e=e: copy(*e, t0 * T, t1 * T) for e in ((wg_hbm, wg_v), (wu_hbm, wu_v))]
    loads = [[copy(x_hbm, x_v, 0, 2 * T)], [gates(9, 11), ups(9, 11)], [copy(x_hbm, x_v, 2 * T, 4 * T), ups(11, 12)],
             [gates(11, 14), ups(12, 14)], [gates(0, 3), ups(0, 3)], [gates(3, 9), ups(3, 9)],
             [copy(wd_hbm, wd_v, 0, F)], [copy(x_hbm, x_v, 4 * T, S)]]
    for c in sum(loads, []):
        c.start()

    def arrive():
        for c in loads.pop(0):
            c.wait()

    def up_tile(k, n, shift):
        c = slice(k * T, (k + 1) * T)
        if n == 26:
            return jnp.concatenate([pltpu.bitcast(ref[pl.ds(FM, F - FM), c], u32) for ref in (wg_v, wu_v)], axis=0)
        return (wg_v, wu_v)[n // 13][pl.ds(pl.multiple_of((n % 13 + shift) * T, T), T), c]

    def down_tile(n, k):
        return wd_v[pl.ds(((k + 18) % 24 if k < 24 else k) * H, H), n * T:(n + 1) * T]

    def weight_sums(table, tile):
        sums = Operands(table, lambda a, b: (1, Rows.of(tile(a, b))), Rows.packed, lambda a, b: (1, Rows.once(tile(a, b))))

        def get(r):
            s, i = table.where[r]
            terms = table.terms[i]
            if not terms:
                return 0, jnp.zeros((H // 2, T), u32)
            if len(terms) == 1 and terms[0][1] not in table.kept:
                return s * terms[0][0], pltpu.bitcast(tile(*terms[0][1]), u32)
            return sums(r)
        return get

    def down_weights():
        half = weight_sums(P["w_down"], down_tile)

        def get(r):
            (s, lo), (s2, hi) = half(2 * r), half(2 * r + 1)
            return s, jnp.concatenate([lo, hi ^ np.uint32(0x80008000) if s * s2 < 0 else hi], axis=0)
        return get

    six_weights = lambda shift: weight_sums(P["w_six"], lambda k, c: up_tile(k, SIX_TILES[c], shift))
    home = [(nine_v, 0), (six_v, 0), (six_v, n6), (six_v, 2 * n6), (down_v, 0)]
    w_sign = {}

    def formed(part, make, where=None):
        ref, base = where or home[part]

        @functools.cache
        def get(r):
            w_sign[part, r], v = make(r)
            ref[base + r] = v
            return w_sign[part, r], pltpu.bitcast(v, bf16)
        return get

    def kept(part):
        return lambda r: (w_sign[2 if part == 3 else part, r], pltpu.bitcast(home[part][0][home[part][1] + r], bf16))

    def x_operands(i, table):
        r0 = pl.multiple_of(i * 2 * T, 2 * T)

        @functools.cache
        def block(m, k):
            v = Rows.of(x_v[pl.ds(r0 + m * T, T), k * T:(k + 1) * T])
            return Rows(v.even * 0.5, v.odd * 0.5) if m else v

        @functools.cache
        def get(d, k):
            return 1, block(1, k) - block(0, k) if d else block(1, k) + block(0, k)
        return Operands(table, get, lambda v: pltpu.bitcast(v.packed(), bf16))

    def gate(chain, tiles, keep):
        other = {}

        def done(i, s, t):
            m, c = divmod(i, len(tiles))
            n = tiles[c]
            if n == 26:
                k, s, t2 = 13, 1, pltpu.roll(t, F - FM, 1)
            elif (m, n % 13) in other:
                k, (s2, t2) = n % 13, other.pop((m, n % 13))
                s *= s2
            else:
                other[m, n % 13] = (s, t)
                return
            keep(m, k, s, (t if m else t * 0.25) * t2)
        return Results(chain, done)

    def h_operands(h, table):
        def tile(d, c):
            s, v = h[1 - d, (c + 9) % 12 if c < 12 else c]
            return s if d else -s, v

        @functools.cache
        def get(d, c):
            if c < 13:
                return tile(d, c)
            (s, a), (s2, b) = tile(d, 12), tile(d, 13)
            a, b = value(a), value(b)
            b = b if s == s2 else -b
            low = lax.broadcasted_iota(jnp.int32, a.shape, 1) < F - FM
            return s, jnp.where(low, a, b) if c == 13 else jnp.where(low, b, a)
        return Operands(table, get, lambda v: v.astype(bf16))

    def out_results(i, groups):
        left = [sum((m1 - m0) * (n1 - n0) for m0, m1, n0, n1 in group) for group in groups]

        def done(e, s, v):
            m, n = divmod(e, 5)
            o_v[i, m * T:(m + 1) * T, n * T:(n + 1) * T] = (v if s > 0 else v * -1.0).astype(bf16)
            j = next(j for j, group in enumerate(groups) for m0, m1, n0, n1 in group if m0 <= m < m1 and n0 <= n < n1)
            left[j] -= 1
            if not left[j]:
                for piece in groups[j]:
                    out_copy(o_v, o_hbm, sem_out, i, *piece).start()
        return Results(P["out"], done)

    def parts(i, x, h, keep, h_table, pieces):
        x_six = lambda r: x(n9 + r)
        return ([(x, gate(P["nine"], NINE_TILES, keep))]
                + [(x_six, gate(P["six"], [n + 3 * g for n in SIX_TILES], keep)) for g in range(3)]
                + [(h_operands(h, h_table), out_results(i, pieces))])

    def multiply(part, pairs, order, weights):
        for e in order:
            r, (left, results) = e // len(pairs), pairs[e % len(pairs)]
            sw, w = weights(r)
            sx, v = left(r)
            dims = (((1,), (int(part < DOWN_PART),)), ((), ()))
            results.add(r, sx * sw, lax.dot_general(v, w, dims, preferred_element_type=f32))

    def to_scratch(i, h, shift=0, copies=(0,)):
        def keep(m, k, s, v):
            h_v[i, m * 14 + k + shift] = v
            for d in copies:
                h[m, k + d] = (s, lambda e=m * 14 + k + d: h_v[i, e])
        return keep

    xs = [x_operands(i, P["x_first"]) for i in range(FIRST)]
    hs = [{} for _ in xs]
    first = [parts(i, xs[i], hs[i], to_scratch(i, hs[i]), P["h_first"], WHOLE) for i in range(FIRST)]
    take = lambda part: [p[part] for p in first]
    arrive()
    weights = formed(0, weight_sums(P["w_nine"], lambda k, c: up_tile(k, NINE_TILES[c], 0)))
    present = ((1, (9, 10, 22, 23)), (2, (9, 10, 22, 23, 24)), (2, NINE_TILES), (2, NINE_TILES))
    for r in AHEAD:
        e = xs[0].table.where[r][1]
        if e not in xs[0].made:
            xs_v[e] = pltpu.bitcast(xs[0](r)[1], u32)
            xs[0].made[e] = (xs[0].made[e][0], pltpu.bitcast(xs_v[e], bf16))
    for order, (pairs, tiles) in zip(FIRST_NINE, present, strict=True):
        assert all(e % 2 < pairs and NINE_TILES[c] in tiles for e in order for c in P["needs"][e // 2])
        arrive()
        multiply(0, take(0), order, weights)
    multiply(1, take(1), FIRST_SIX[0], formed(1, six_weights(0)))

    def two_more(g, carry):
        tiles = [n + 3 for n in SIX_TILES]
        pairs = [(first[i][2][0], gate(P["six"], tiles, to_scratch(i, hs[i], 3 * g, (0, 3)))) for i in range(FIRST)]
        multiply(2, pairs, FIRST_SIX[1], formed(2, six_weights(3 + 3 * g), (six_v, (1 + g) * n6)))
        return carry

    arrive()
    lax.fori_loop(0, 2, two_more, 0)
    arrive()
    multiply(DOWN_PART, take(DOWN_PART), FIRST_DOWN, formed(DOWN_PART, down_weights()))

    def body(it, carry):
        for u in range(UNROLL):
            i, h = FIRST + it * UNROLL + u, {}
            here = parts(i, x_operands(i, P["x"]), h, lambda m, k, s, v, h=h: h.update({(m, k): (s, v)}), P["h"],
                         PIECES if u == UNROLL - 1 else WHOLE)
            for part, order in enumerate(LOOP[u]):
                multiply(part, [here[part]], order, kept(part))
        return carry

    arrive()
    lax.fori_loop(0, (S // (2 * T) - FIRST) // UNROLL, body, 0)


@jax.jit
def pallas_standalone__glu_gated_bilinear__prompt_kernel(x, w_gate, w_up, w_down):
    B, S, D = x.shape
    F = w_gate.shape[1]
    assert (D, F) == (640, 1728) and (B * S // (2 * T) - FIRST) % UNROLL == 0 and B * S % (2 * T) == 0
    vmem = pltpu.VMEM
    out = pl.pallas_call(
        kernel,
        in_specs=[pl.BlockSpec(memory_space=pl.ANY)] * 4,
        out_specs=pl.BlockSpec(memory_space=pl.ANY),
        out_shape=jax.ShapeDtypeStruct((B * S, D), x.dtype),
        scratch_shapes=[
            vmem((B * S // (2 * T), 2 * T, D), bf16), pltpu.SemaphoreType.DMA((1,)),
            vmem((B * S, D), bf16), vmem((F, D), bf16), vmem((F, D), bf16), vmem((F, D), bf16),
            vmem((len(plan()["x_first"].terms), H, T), u32), vmem((FIRST, 28, T, T), f32),
            *[vmem((n * len(plan()[part].where), H, T), u32) for n, part in ((1, "nine"), (3, "six"), (1, "out"))],
        ],
        compiler_params=pltpu.CompilerParams(vmem_limit_bytes=100 * 2**20),
    )(x.reshape(B * S, D), w_gate.T, w_up.T, w_down)
    return out.reshape(B, S, D)
```
